```python
import os as _os
_os.environ.setdefault("JAX_PLATFORMS", "cpu")
import jax
import jax.numpy as jnp

def _softmax(x, axis=-1):
    return jax.nn.softmax(x, axis=axis)
def _gelu(x):
    return jax.nn.gelu(x, approximate=True)
def _silu(x):
    return jax.nn.silu(x)
def _sigmoid(x):
    return jax.nn.sigmoid(x)
def _layernorm(x, axis=-1, eps=1e-5):
    m = jnp.mean(x, axis=axis, keepdims=True)
    v = jnp.var(x, axis=axis, keepdims=True)
    return (x - m) / jnp.sqrt(v + eps)
def _scatter_add(tgt, idx, src, axis=0):
    return tgt.at[idx].add(src)
def _segment_sum(src, seg, n):
    return jax.ops.segment_sum(src, seg, n)
class _Rng:
    def __init__(self, key):
        self._k = key
    def _next(self):
        self._k, sub = jax.random.split(self._k)
        return sub
    def normal(self, shape):
        return jax.random.normal(self._next(), shape, dtype=jnp.bfloat16)
    def randint(self, lo, hi, shape):
        return jax.random.randint(self._next(), shape, lo, hi, dtype=jnp.int32)
    def uniform(self, shape, lo=0.0, hi=1.0):
        return jax.random.uniform(self._next(), shape, jnp.bfloat16, lo, hi)
    def permutation(self, n):
        return jax.random.permutation(self._next(), n)


kernel_name = 'interleave_layers__sliding_block__dense_activation_gelu__prompt'

def setup_inputs():
    _rng = _Rng(jax.random.key(int.from_bytes(__import__("os").urandom(4), "little")))
    _w = (lambda a: (lambda t: t.astype(jnp.bfloat16) if jnp.issubdtype(t.dtype, jnp.floating) else t)(jnp.asarray(a)))
    def _A_setup():
        B, S, D = 1, 2048, 640
        return {
            "x": _w((lambda *s: _rng.normal(s) * 0.05)(B, S, D)),
            "wqkv": _w((lambda *s: _rng.normal(s) * 0.05)(D, 3 * D)),
            "wo": _w((lambda *s: _rng.normal(s) * 0.05)(D, D)),
        }
    _A_in = _A_setup()

    def _B_setup():
        B, S, D, F = 1, 2048, 640, 1728
        return {
            "x": _w((lambda *s: _rng.normal(s) * 0.05)(B, S, D)),
            "w1": _w((lambda *s: _rng.normal(s) * 0.8)(D, F) * (D ** -0.5)),
            "b1": _w((lambda *s: _rng.normal(s) * 0.8)(F) * 0.01),
            "w2": _w((lambda *s: _rng.normal(s) * 0.8)(F, D) * (F ** -0.5)),
            "b2": _w((lambda *s: _rng.normal(s) * 0.8)(D) * 0.01),
        }
    _B_in = _B_setup()

    return {
        "A_x": _A_in["x"],
        "A_wqkv": _A_in["wqkv"],
        "A_wo": _A_in["wo"],
        "B_x": _B_in["x"],
        "B_w1": _B_in["w1"],
        "B_b1": _B_in["b1"],
        "B_w2": _B_in["w2"],
        "B_b2": _B_in["b2"],
    }

def reference(A_x, A_wqkv, A_wo, B_x, B_w1, B_b1, B_w2, B_b2):
    def _A_ref(x, wqkv, wo):
        B, S, D = x.shape
        H = 32; Dh = D // H; W = 256
        qkv = (lambda x, *d: x.transpose(*d))((x @ wqkv).reshape(B, S, 3, H, Dh), 2, 0, 3, 1, 4)
        q, k, v = qkv[0], qkv[1], qkv[2]
        scores = jnp.einsum("bhqd,bhkd->bhqk", q, k) * (Dh ** -0.5)
        idx = jnp.arange(S)
        mask = (idx[:, None] - idx[None, :] >= 0) & (idx[:, None] - idx[None, :] < W)
        scores = jnp.where(mask[None, None], scores, -1e9)
        p = _softmax(scores, axis=-1)
        o = jnp.einsum("bhqk,bhkd->bhqd", p, v)
        return (lambda x, *d: x.transpose(*d))(o, 0, 2, 1, 3).reshape(B, S, D) @ wo

    def _B_ref(x, w1, b1, w2, b2):
        h = jnp.einsum("bsd,df->bsf", x, w1) + b1
        h = _gelu(h)
        return jnp.einsum("bsf,fd->bsd", h, w2) + b2

    x = A_x
    x = x + _A_ref(_layernorm(x, axis=-1), A_wqkv, A_wo)
    x = x + _B_ref(_layernorm(x, axis=-1), B_w1, B_b1, B_w2, B_b2)
    x = x + _A_ref(_layernorm(x, axis=-1), A_wqkv, A_wo)
    x = x + _B_ref(_layernorm(x, axis=-1), B_w1, B_b1, B_w2, B_b2)
    return x
```

```python
import math
import jax
import jax.numpy as jnp
from jax import lax
import jax.experimental.pallas as pl
import jax.experimental.pallas.tpu as pltpu

S, D, H, DH, W, F = 2048, 640, 32, 20, 256, 1728
T = 128
R = 256
NB = S // R
NT = (((1,), (1,)), ((), ()))
BF = jnp.bfloat16
F32 = jnp.float32
QSCALE = (DH ** -0.5) * math.log2(math.e)


def _ln(x):
    m = jnp.mean(x, axis=-1, keepdims=True)
    c = x - m
    v = jnp.mean(c * c, axis=-1, keepdims=True)
    return c * lax.rsqrt(v + 1e-5)


def _head_tile(h):
    lo, hi = DH * h, DH * h + DH - 1
    if lo // 128 == hi // 128:
        return lo // 128, lo % 128
    t = (lo - 64) // 128
    return 5 + t, lo - 64 - 128 * t


def _kernel(x_ref, wqkv_ref, wo_ref, w1_ref, b1_ref, w2_ref, b2_ref, o_ref,
            xs, q_s, k_s, vt_s, wvt_s, ot_s):
    wvt_s[...] = wqkv_ref[:, 2 * D:].astype(F32).T.astype(BF)
    k_s[:, 0:W, :] = jnp.zeros((9, W, 128), BF)
    vt_s[:, :, 0:W] = jnp.zeros((H, 32, W), BF)

    def qkv(j, first):
        r0 = pl.multiple_of(j * R, R)
        if first:
            x = x_ref[pl.ds(r0, R), :].astype(F32)
            xs[pl.ds(r0, R), :] = x
        else:
            x = xs[pl.ds(r0, R), :]
        xn = _ln(x).astype(BF)
        q = jnp.dot(xn, wqkv_ref[:, 0:D], preferred_element_type=F32) * QSCALE
        k = jnp.dot(xn, wqkv_ref[:, D:2 * D], preferred_element_type=F32)
        for t in range(9):
            c0 = 128 * t if t < 5 else 64 + 128 * (t - 5)
            q_s[t, pl.ds(r0, R), :] = q[:, c0:c0 + 128].astype(BF)
            k_s[t, pl.ds(r0 + W, R), :] = k[:, c0:c0 + 128].astype(BF)
        vt = lax.dot_general(wvt_s[...], xn, NT, preferred_element_type=F32)
        vt = jnp.concatenate([vt, jnp.zeros((8, R), F32)], axis=0)
        row = lax.broadcasted_iota(jnp.int32, (32, R), 0)
        for h in range(H):
            w0 = 40 * (h // 2) + 16 * (h % 2)
            one = 0 if h % 2 else 24
            blk = jnp.where(row == one, 1.0, vt[w0:w0 + 32, :])
            vt_s[h, :, pl.ds(r0 + W, R)] = blk.astype(BF)

    def attn_tile(i, half, edge):
        q0 = pl.multiple_of(i * T, T)
        kk = lax.broadcasted_iota(jnp.int32, (T, T), 0)
        qq = lax.broadcasted_iota(jnp.int32, (T, T), 1)
        upper = kk > qq
        if edge:
            ba = jnp.where(i >= 2, 0.0, -1e30).astype(F32)
            bb = jnp.where(i >= 1, 0.0, -1e30).astype(F32)
        lane = lax.broadcasted_iota(jnp.int32, (T, 128), 1)
        sub = lax.broadcasted_iota(jnp.int32, (8, T), 0)
        prev = None
        for h in range(H):
            t, off = _head_tile(h)
            qt = q_s[t, pl.ds(q0, T), :]
            qm = jnp.where((lane >= off) & (lane < off + DH), qt, jnp.zeros_like(qt))
            kt = k_s[t, pl.ds(q0, 3 * T), :]
            s = lax.dot_general(kt, qm, NT, preferred_element_type=F32)
            sa, sb, sc = s[0:T], s[T:2 * T], s[2 * T:]
            if edge:
                sa = sa + ba
                sb = sb + bb
            sm = jnp.where(upper, sa, sc)
            mx = jnp.max(jnp.maximum(sm, sb), axis=0, keepdims=True)
            pm = jnp.exp2(sm - mx)
            pb = jnp.exp2(sb - mx).astype(BF)
            pa = jnp.where(upper, pm, 0.0).astype(BF)
            pc = jnp.where(upper, 0.0, pm).astype(BF)
            p = jnp.concatenate([pa, pb, pc], axis=0)
            o = jnp.dot(vt_s[h, :, pl.ds(q0, 3 * T)], p, preferred_element_type=F32)
            if h % 2 == 0:
                prev = o[0:24] * (1.0 / o[24:25])
            else:
                on = o * (1.0 / o[0:1])
                mid = jnp.where(sub < 4, prev[16:24], on[0:8])
                b0 = 20 * (h - 1)
                ot_s[b0:b0 + 40, pl.ds(half * T, T)] = jnp.concatenate(
                    [prev[0:16], mid, on[8:24]], axis=0)

    def attn(j, edge):
        for half in range(2):
            attn_tile(2 * j + half, half, edge)

    def ffn(j, last):
        r0 = pl.multiple_of(j * R, R)
        o = ot_s[...].T.astype(BF)
        x = xs[pl.ds(r0, R), :] + jnp.dot(o, wo_ref[...], preferred_element_type=F32)
        xn = _ln(x).astype(BF)
        hh = jnp.dot(xn, w1_ref[...], preferred_element_type=F32) + b1_ref[...].astype(F32)
        g = jax.nn.gelu(hh, approximate=True).astype(BF)
        y = x + jnp.dot(g, w2_ref[...], preferred_element_type=F32) + b2_ref[...].astype(F32)
        if last:
            o_ref[pl.ds(r0, R), :] = y.astype(o_ref.dtype)
        else:
            xs[pl.ds(r0, R), :] = y

    for layer in range(2):
        def p1(j, c):
            qkv(j, layer == 0)
            return c
        lax.fori_loop(0, NB, p1, 0)
        attn(0, True)
        ffn(0, layer == 1)

        def p2(j, c):
            attn(j, False)
            ffn(j, layer == 1)
            return c
        lax.fori_loop(1, NB, p2, 0)


@jax.jit
def pallas_interleave_layers__sliding_block__dense_activation_gelu__prompt_kernel(
    A_x, A_wqkv, A_wo, B_x, B_w1, B_b1, B_w2, B_b2,
):
    vm = pl.BlockSpec(memory_space=pltpu.VMEM)
    out = pl.pallas_call(
        _kernel,
        out_shape=jax.ShapeDtypeStruct((S, D), A_x.dtype),
        in_specs=[vm] * 7,
        out_specs=vm,
        scratch_shapes=[
            pltpu.VMEM((S, D), F32),
            pltpu.VMEM((9, S, 128), BF),
            pltpu.VMEM((9, S + W, 128), BF),
            pltpu.VMEM((H, 32, S + W), BF),
            pltpu.VMEM((D, D), BF),
            pltpu.VMEM((D, R), F32),
        ],
        compiler_params=pltpu.CompilerParams(vmem_limit_bytes=100 * 1024 * 1024),
    )(A_x.reshape(S, D), A_wqkv, A_wo, B_w1, B_b1.reshape(1, F), B_w2, B_b2.reshape(1, D))
    return out.reshape(1, S, D)
```

```python
import math
import jax
import jax.numpy as jnp
from jax import lax
import jax.experimental.pallas as pl
import jax.experimental.pallas.tpu as pltpu

S, D, H, DH, W, F = 2048, 640, 32, 20, 256, 1728
T = 128
R = 256
NB = S // R
NT = (((1,), (1,)), ((), ()))
BF = jnp.bfloat16
F32 = jnp.float32
I32 = jnp.int32
_pk = lambda v: pltpu.bitcast(v.astype(BF), I32)
_up = lambda v: pltpu.bitcast(v, BF)
QSCALE = (DH ** -0.5) * math.log2(math.e)


def _ln(x):
    m = jnp.mean(x, axis=-1, keepdims=True)
    c = x - m
    v = jnp.mean(c * c, axis=-1, keepdims=True)
    return c * lax.rsqrt(v + 1e-5)


def _head_tile(h):
    lo, hi = DH * h, DH * h + DH - 1
    if lo // 128 == hi // 128:
        return lo // 128, lo % 128
    t = (lo - 64) // 128
    return 5 + t, lo - 64 - 128 * t


def _kernel(x_h, wqkv_h, wo_h, w1_h, b1_ref, w2_h, b2_ref, o_h,
            xs, q_s, k_s, vt_s, wvt_s, ot_s, x_ref, wqkv_ref, wo_ref, w1_ref, w2_ref, o_ref, sems):
    cps = [pltpu.make_async_copy(a, b, sems.at[n]) for n, (a, b) in enumerate(
        [(wqkv_h, wqkv_ref), (x_h, x_ref), (wo_h, wo_ref), (w1_h, w1_ref), (w2_h, w2_ref)])]
    for c in cps:
        c.start()
    HALF = S // 2
    ocp = [pltpu.make_async_copy(o_ref.at[pl.ds(u * HALF, HALF)], o_h.at[pl.ds(u * HALF, HALF)], sems.at[5 + u])
           for u in range(2)]
    cps[0].wait()
    wvt_s[...] = wqkv_ref[:, 2 * D:].astype(F32).T.astype(BF)
    k_s[:, 0:W // 2, :] = jnp.zeros((9, W // 2, 128), I32)
    vt_s[:, :, 0:W] = jnp.zeros((H, 16, W), I32)

    cps[1].wait()

    def qkv(j, first):
        r0 = pl.multiple_of(j * R, R)
        if first:
            x = x_ref[pl.ds(r0, R), :].astype(F32)
            xs[pl.ds(r0, R), :] = x
        else:
            x = xs[pl.ds(r0, R), :]
        xn = _ln(x).astype(BF)
        q = jnp.dot(xn, wqkv_ref[:, 0:D], preferred_element_type=F32) * QSCALE
        k = jnp.dot(xn, wqkv_ref[:, D:2 * D], preferred_element_type=F32)
        for t in range(9):
            c0 = 128 * t if t < 5 else 64 + 128 * (t - 5)
            q_s[t, pl.ds(pl.multiple_of(r0 // 2, R // 2), R // 2), :] = _pk(q[:, c0:c0 + 128])
            k_s[t, pl.ds(pl.multiple_of(r0 // 2, R // 2) + W // 2, R // 2), :] = _pk(k[:, c0:c0 + 128])
        vt = lax.dot_general(wvt_s[...], xn, NT, preferred_element_type=F32)
        vt = jnp.concatenate([vt, jnp.zeros((8, R), F32)], axis=0)
        row = lax.broadcasted_iota(jnp.int32, (32, R), 0)
        for h in range(H):
            w0 = 40 * (h // 2) + 16 * (h % 2)
            one = 0 if h % 2 else 24
            blk = jnp.where(row == one, 1.0, vt[w0:w0 + 32, :])
            vt_s[h, :, pl.ds(r0 + W, R)] = _pk(blk)

    def attn_tile(i, half, edge):
        q0 = pl.multiple_of(i * T, T)
        kk = lax.broadcasted_iota(jnp.int32, (T, T), 0)
        qq = lax.broadcasted_iota(jnp.int32, (T, T), 1)
        upper = kk > qq
        if edge:
            ba = jnp.where(i >= 2, 0.0, -1e30).astype(F32)
            bb = jnp.where(i >= 1, 0.0, -1e30).astype(F32)
        lane = lax.broadcasted_iota(jnp.int32, (T, 128), 1)
        sub = lax.broadcasted_iota(jnp.int32, (8, T), 0)
        q2 = pl.multiple_of(i * (T // 2), T // 2)

        def scores(h):
            t, off = _head_tile(h)
            qt = _up(q_s[t, pl.ds(q2, T // 2), :])
            qm = jnp.where((lane >= off) & (lane < off + DH), qt, jnp.zeros_like(qt))
            kt = _up(k_s[t, pl.ds(q2, 3 * T // 2), :])
            return lax.dot_general(kt, qm, NT, preferred_element_type=F32)

        def probs(s):
            sa, sb, sc = s[0:T], s[T:2 * T], s[2 * T:]
            if edge:
                sa = sa + ba
                sb = sb + bb
            sm = jnp.where(upper, sa, sc)
            mx = jnp.max(jnp.maximum(sm, sb), axis=0, keepdims=True)
            pm = jnp.exp2(sm - mx)
            pb = jnp.exp2(sb - mx).astype(BF)
            pa = jnp.where(upper, pm, 0.0).astype(BF)
            pc = jnp.where(upper, 0.0, pm).astype(BF)
            return jnp.concatenate([pa, pb, pc], axis=0)

        def pv(h, p):
            return jnp.dot(_up(vt_s[h, :, pl.ds(q0, 3 * T)]), p, preferred_element_type=F32)

        G = 4
        ss = [scores(h) for h in range(G)]
        for g0 in range(0, H, G):
            ps = [probs(s) for s in ss]
            if g0 + G < H:
                ss = [scores(h) for h in range(g0 + G, g0 + 2 * G)]
            os_ = [pv(g0 + u, ps[u]) for u in range(G)]
            for u in range(0, G, 2):
                oe, oo = os_[u], os_[u + 1]
                prev = oe[0:24] * (1.0 / oe[24:25])
                on = oo * (1.0 / oo[0:1])
                mid = jnp.where(sub < 4, prev[16:24], on[0:8])
                b0 = 20 * (g0 + u)
                ot_s[(i // 2) % 2, b0:b0 + 40, pl.ds(half * T, T)] = jnp.concatenate(
                    [prev[0:16], mid, on[8:24]], axis=0)

    def attn(j, edge):
        for half in range(2):
            attn_tile(2 * j + half, half, edge)

    def ffn(j, last):
        r0 = pl.multiple_of(j * R, R)
        o = ot_s[j % 2].T.astype(BF)
        x = xs[pl.ds(r0, R), :] + jnp.dot(o, wo_ref[...], preferred_element_type=F32)
        xn = _ln(x).astype(BF)
        hh = lax.dot_general(xn, w1_ref[...], NT, preferred_element_type=F32) + b1_ref[...].astype(F32)
        g = jax.nn.gelu(hh, approximate=True).astype(BF)
        y = x + jnp.dot(g, w2_ref[...], preferred_element_type=F32) + b2_ref[...].astype(F32)
        if last:
            o_ref[pl.ds(r0, R), :] = y.astype(o_ref.dtype)
        else:
            xs[pl.ds(r0, R), :] = y

    for layer in range(2):
        def p1(j, c):
            qkv(j, layer == 0)
            return c
        lax.fori_loop(0, NB, p1, 0)
        attn(0, True)
        if layer == 0:
            for c in cps[2:]:
                c.wait()

        def p2(j, c):
            ffn(j - 1, layer == 1)
            attn(j, False)
            return c
        if layer == 0:
            lax.fori_loop(1, NB, p2, 0)
        else:
            lax.fori_loop(1, NB // 2 + 1, p2, 0)
            ocp[0].start()
            lax.fori_loop(NB // 2 + 1, NB, p2, 0)
        ffn(NB - 1, layer == 1)
    ocp[1].start()
    ocp[0].wait()
    ocp[1].wait()


@jax.jit
def pallas_interleave_layers__sliding_block__dense_activation_gelu__prompt_kernel(
    A_x, A_wqkv, A_wo, B_x, B_w1, B_b1, B_w2, B_b2,
):
    hb = pl.BlockSpec(memory_space=pl.ANY)
    vm = pl.BlockSpec(memory_space=pltpu.VMEM)
    out = pl.pallas_call(
        _kernel,
        out_shape=jax.ShapeDtypeStruct((S, D), A_x.dtype),
        in_specs=[hb, hb, hb, hb, vm, hb, vm],
        out_specs=hb,
        scratch_shapes=[
            pltpu.VMEM((S, D), F32),
            pltpu.VMEM((9, S // 2, 128), I32),
            pltpu.VMEM((9, (S + W) // 2, 128), I32),
            pltpu.VMEM((H, 16, S + W), I32),
            pltpu.VMEM((D, D), BF),
            pltpu.VMEM((2, D, R), F32),
            pltpu.VMEM((S, D), BF), pltpu.VMEM((D, 3 * D), BF), pltpu.VMEM((D, D), BF),
            pltpu.VMEM((F, D), BF), pltpu.VMEM((F, D), BF), pltpu.VMEM((S, D), BF),
            pltpu.SemaphoreType.DMA((7,)),
        ],
        compiler_params=pltpu.CompilerParams(vmem_limit_bytes=100 * 1024 * 1024),
    )(A_x.reshape(S, D), A_wqkv, A_wo, B_w1.T, B_b1.reshape(1, F), B_w2, B_b2.reshape(1, D))
    return out.reshape(1, S, D)
```

```python
import math
import jax
import jax.numpy as jnp
from jax import lax
import jax.experimental.pallas as pl
import jax.experimental.pallas.tpu as pltpu

S, D, H, DH, W, F = 2048, 640, 32, 20, 256, 1728
T = 128
R = 256
NB = S // R
FC = 128
NC = 128
NT = (((1,), (1,)), ((), ()))
BF = jnp.bfloat16
F32 = jnp.float32
I32 = jnp.int32
_pk = lambda v: pltpu.bitcast(v.astype(BF), I32)
_up = lambda v: pltpu.bitcast(v, BF)
QSCALE = (DH ** -0.5) * math.log2(math.e)


def _ln(x):
    m = jnp.mean(x, axis=-1, keepdims=True)
    c = x - m
    v = jnp.mean(c * c, axis=-1, keepdims=True)
    return c * lax.rsqrt(v + 1e-5)


def _head_tile(h):
    lo, hi = DH * h, DH * h + DH - 1
    if lo // 128 == hi // 128:
        return lo // 128, lo % 128
    t = (lo - 64) // 128
    return 5 + t, lo - 64 - 128 * t


def _kernel(x_h, wqkv_h, wo_h, w1_h, b1_ref, w2_h, b2_ref, o_h,
            xs, q_s, k_s, vt_s, wvt_s, ot_s, x_ref, wqkv_ref, wo_ref, w1_ref, w2_ref, o_ref, g_s, sems):
    cps = [pltpu.make_async_copy(a, b, sems.at[n]) for n, (a, b) in enumerate(
        [(wqkv_h, wqkv_ref), (x_h.at[0:R], x_ref.at[0:R]), (wo_h, wo_ref), (w1_h, w1_ref), (w2_h, w2_ref)])]
    xcp = [cps[1],
           pltpu.make_async_copy(x_h.at[R:2 * R], x_ref.at[R:2 * R], sems.at[7]),
           pltpu.make_async_copy(x_h.at[2 * R:S], x_ref.at[2 * R:S], sems.at[8])]
    for c in cps[:2] + xcp[1:] + cps[2:]:
        c.start()
    HALF = S // 2
    ocp = [pltpu.make_async_copy(o_ref.at[pl.ds(u * HALF, HALF)], o_h.at[pl.ds(u * HALF, HALF)], sems.at[5 + u])
           for u in range(2)]
    cps[0].wait()
    wvt_s[...] = wqkv_ref[:, 2 * D:].astype(F32).T.astype(BF)
    k_s[:, 0:W // 2, :] = jnp.zeros((9, W // 2, 128), I32)
    vt_s[:, :, 0:W] = jnp.zeros((H, 16, W), I32)


    def qkv(j, first):
        r0 = j * R if isinstance(j, int) else pl.multiple_of(j * R, R)
        rh = j * (R // 2) if isinstance(j, int) else pl.multiple_of(j * (R // 2), R // 2)
        if first:
            x = x_ref[pl.ds(r0, R), :].astype(F32)
            xs[pl.ds(r0, R), :] = x
        else:
            x = xs[pl.ds(r0, R), :]
        xn = _ln(x).astype(BF)
        q = jnp.dot(xn, wqkv_ref[:, 0:D], preferred_element_type=F32) * QSCALE
        for t in range(9):
            c0 = 128 * t if t < 5 else 64 + 128 * (t - 5)
            q_s[t, pl.ds(rh, R // 2), :] = _pk(q[:, c0:c0 + 128])
        yield
        yield
        k = jnp.dot(xn, wqkv_ref[:, D:2 * D], preferred_element_type=F32)
        for t in range(9):
            c0 = 128 * t if t < 5 else 64 + 128 * (t - 5)
            k_s[t, pl.ds(rh + W // 2, R // 2), :] = _pk(k[:, c0:c0 + 128])
        yield
        yield
        vt = lax.dot_general(wvt_s[...], xn, NT, preferred_element_type=F32)
        vt = jnp.concatenate([vt, jnp.zeros((8, R), F32)], axis=0)
        row = lax.broadcasted_iota(jnp.int32, (32, R), 0)
        for h in range(H):
            w0 = 40 * (h // 2) + 16 * (h % 2)
            one = 0 if h % 2 else 24
            blk = jnp.where(row == one, 1.0, vt[w0:w0 + 32, :])
            vt_s[h, :, pl.ds(r0 + W, R)] = _pk(blk)

    def attn_tile(i, half, edge):
        q0 = i * T if edge else pl.multiple_of(i * T, T)
        sk = (2 - i) if edge else 0
        kk = lax.broadcasted_iota(jnp.int32, (T, T), 0)
        qq = lax.broadcasted_iota(jnp.int32, (T, T), 1)
        upper = kk > qq
        lane = lax.broadcasted_iota(jnp.int32, (T, 128), 1)
        sub = lax.broadcasted_iota(jnp.int32, (8, T), 0)
        q2 = i * (T // 2) if edge else pl.multiple_of(i * (T // 2), T // 2)

        def scores(h):
            t, off = _head_tile(h)
            qt = _up(q_s[t, pl.ds(q2, T // 2), :])
            qm = jnp.where((lane >= off) & (lane < off + DH), qt, jnp.zeros_like(qt))
            kt = _up(k_s[t, pl.ds(q2 + sk * T // 2, (3 - sk) * T // 2), :])
            return lax.dot_general(kt, qm, NT, preferred_element_type=F32)

        def probs(s):
            if edge:
                sc = jnp.where(upper, -1e9, s[-T:])
                sall = sc if sk == 2 else jnp.concatenate([s[0:T], sc], axis=0)
                return jnp.exp2(sall - jnp.max(sall, axis=0, keepdims=True)).astype(BF)
            sa, sb, sc = s[0:T], s[T:2 * T], s[2 * T:]
            sm = jnp.where(upper, sa, sc)
            mx = jnp.max(jnp.maximum(sm, sb), axis=0, keepdims=True)
            pm = jnp.exp2(sm - mx)
            pb = jnp.exp2(sb - mx).astype(BF)
            pa = jnp.where(upper, pm, 0.0).astype(BF)
            pc = jnp.where(upper, 0.0, pm).astype(BF)
            return jnp.concatenate([pa, pb, pc], axis=0)

        def pv(h, p):
            return jnp.dot(_up(vt_s[h, :, pl.ds(q0 + sk * T, (3 - sk) * T)]), p, preferred_element_type=F32)

        G = 4
        ss = [scores(h) for h in range(G)]
        for g0 in range(0, H, G):
            ps = [probs(s) for s in ss]
            if g0 + G < H:
                ss = [scores(h) for h in range(g0 + G, g0 + 2 * G)]
            os_ = [pv(g0 + u, ps[u]) for u in range(G)]
            yield
            for u in range(0, G, 2):
                oe, oo = os_[u], os_[u + 1]
                prev = oe[0:24] * (1.0 / oe[24:25])
                on = oo * (1.0 / oo[0:1])
                mid = jnp.where(sub < 4, prev[16:24], on[0:8])
                b0 = 20 * (g0 + u)
                ot_s[(i // 2) % 2, b0:b0 + 40, pl.ds(half * T, T)] = jnp.concatenate(
                    [prev[0:16], mid, on[8:24]], axis=0)

    def attn(j, edge):
        for half in range(2):
            yield from attn_tile(2 * j + half, half, edge)

    def run(*gens):
        gens = list(gens)
        while gens:
            for g in list(gens):
                try:
                    next(g)
                except StopIteration:
                    gens.remove(g)

    def ffn(j, last):
        r0 = j * R if isinstance(j, int) else pl.multiple_of(j * R, R)
        o = ot_s[j % 2].T.astype(BF)
        x = xs[pl.ds(r0, R), :] + jnp.dot(o, wo_ref[...], preferred_element_type=F32)
        xn = _ln(x).astype(BF)
        xs[pl.ds(r0, R), :] = x
        yield
        for c0 in range(0, F, FC):
            c1 = min(F, c0 + FC)
            hh = lax.dot_general(xn, w1_ref[c0:c1, :], NT, preferred_element_type=F32)
            hh = hh + b1_ref[:, c0:c1].astype(F32)
            g_s[:, c0:c1] = _pk(jax.nn.gelu(hh, approximate=True))
            yield
        for c0 in range(0, D, NC):
            c1 = c0 + NC
            y = (xs[pl.ds(r0, R), c0:c1] + b2_ref[:, c0:c1].astype(F32)
                 + jnp.dot(_up(g_s[...]), w2_ref[:, c0:c1], preferred_element_type=F32))
            if last:
                o_ref[pl.ds(r0, R), c0:c1] = y.astype(o_ref.dtype)
            else:
                xs[pl.ds(r0, R), c0:c1] = y
            yield

    for layer in range(2):
        if layer == 0:
            xcp[0].wait()
            run(qkv(0, True))
            xcp[1].wait()
        else:
            run(ffn(NB - 1, False), qkv(0, False))
        run(attn(0, True), qkv(1, layer == 0))
        if layer == 0:
            xcp[2].wait()

        def p1(j, c):
            run(qkv(j, layer == 0))
            return c
        lax.fori_loop(2, NB, p1, 0)
        if layer == 0:
            for c in cps[2:]:
                c.wait()

        def p2(j, c):
            run(attn(j, False), ffn(j - 1, layer == 1))
            return c
        if layer == 0:
            lax.fori_loop(1, NB, p2, 0)
        else:
            lax.fori_loop(1, NB // 2 + 1, p2, 0)
            ocp[0].start()
            lax.fori_loop(NB // 2 + 1, NB, p2, 0)
            run(ffn(NB - 1, True))
    ocp[1].start()
    ocp[0].wait()
    ocp[1].wait()


@jax.jit
def pallas_interleave_layers__sliding_block__dense_activation_gelu__prompt_kernel(
    A_x, A_wqkv, A_wo, B_x, B_w1, B_b1, B_w2, B_b2,
):
    hb = pl.BlockSpec(memory_space=pl.ANY)
    vm = pl.BlockSpec(memory_space=pltpu.VMEM)
    out = pl.pallas_call(
        _kernel,
        out_shape=jax.ShapeDtypeStruct((S, D), A_x.dtype),
        in_specs=[hb, hb, hb, hb, vm, hb, vm],
        out_specs=hb,
        scratch_shapes=[
            pltpu.VMEM((S, D), F32),
            pltpu.VMEM((9, S // 2, 128), I32),
            pltpu.VMEM((9, (S + W) // 2, 128), I32),
            pltpu.VMEM((H, 16, S + W), I32),
            pltpu.VMEM((D, D), BF),
            pltpu.VMEM((2, D, R), F32),
            pltpu.VMEM((S, D), BF), pltpu.VMEM((D, 3 * D), BF), pltpu.VMEM((D, D), BF),
            pltpu.VMEM((F, D), BF), pltpu.VMEM((F, D), BF), pltpu.VMEM((S, D), BF),
            pltpu.VMEM((R // 2, F), I32),
            pltpu.SemaphoreType.DMA((9,)),
        ],
        compiler_params=pltpu.CompilerParams(vmem_limit_bytes=100 * 1024 * 1024),
    )(A_x.reshape(S, D), A_wqkv, A_wo, B_w1.T, B_b1.reshape(1, F), B_w2, B_b2.reshape(1, D))
    return out.reshape(1, S, D)
```

```python
import math
import jax
import jax.numpy as jnp
from jax import lax
import jax.experimental.pallas as pl
import jax.experimental.pallas.tpu as pltpu

S, D, H, DH, W, F = 2048, 640, 32, 20, 256, 1728
T = 128
R = 256
NB = S // R
FC = 128
NC = 128
NT = (((1,), (1,)), ((), ()))
BF = jnp.bfloat16
F32 = jnp.float32
I32 = jnp.int32
_pk = lambda v: pltpu.bitcast(v.astype(BF), I32)
_up = lambda v: pltpu.bitcast(v, BF)
QSCALE = (DH ** -0.5) * math.log2(math.e)


def _ln(x):
    m = jnp.mean(x, axis=-1, keepdims=True)
    c = x - m
    v = jnp.mean(c * c, axis=-1, keepdims=True)
    return c * lax.rsqrt(v + 1e-5)


def _head_tile(h):
    lo, hi = DH * h, DH * h + DH - 1
    if lo // 128 == hi // 128:
        return lo // 128, lo % 128
    t = (lo - 64) // 128
    return 5 + t, lo - 64 - 128 * t


def _kernel(x_h, wqkv_h, wo_h, w1_h, b1_ref, w2_h, b2_ref, o_h,
            xs, q_s, k_s, vt_s, wvt_s, ot_s, x_ref, wqkv_ref, wo_ref, w1_ref, w2_ref, o_ref, g_s, sems):
    cps = [pltpu.make_async_copy(a, b, sems.at[n]) for n, (a, b) in enumerate(
        [(wqkv_h, wqkv_ref), (x_h.at[0:R], x_ref.at[0:R]), (wo_h, wo_ref), (w1_h, w1_ref), (w2_h, w2_ref)])]
    xcp = [cps[1],
           pltpu.make_async_copy(x_h.at[R:2 * R], x_ref.at[R:2 * R], sems.at[7]),
           pltpu.make_async_copy(x_h.at[2 * R:S], x_ref.at[2 * R:S], sems.at[8])]
    for c in cps[:2] + xcp[1:] + cps[2:]:
        c.start()
    HALF = S // 2
    ocp = [pltpu.make_async_copy(o_ref.at[pl.ds(u * HALF, HALF)], o_h.at[pl.ds(u * HALF, HALF)], sems.at[5 + u])
           for u in range(2)]
    cps[0].wait()
    wvt_s[...] = wqkv_ref[:, 2 * D:].astype(F32).T.astype(BF)
    k_s[:, 0:W // 2, :] = jnp.zeros((18, W // 2, 128), I32)
    vt_s[:, :, 0:W] = jnp.zeros((H, 16, W), I32)


    def qkv(j, first):
        r0 = j * R if isinstance(j, int) else pl.multiple_of(j * R, R)
        rh = j * (R // 2) if isinstance(j, int) else pl.multiple_of(j * (R // 2), R // 2)
        if first:
            x = x_ref[pl.ds(r0, R), :].astype(F32)
            xs[pl.ds(r0, R), :] = x
        else:
            x = xs[pl.ds(r0, R), :]
        xn = _ln(x).astype(BF)
        q = jnp.dot(xn, wqkv_ref[:, 0:D], preferred_element_type=F32) * QSCALE
        for t in range(9):
            c0 = 128 * t if t < 5 else 64 + 128 * (t - 5)
            q_s[t, pl.ds(rh, R // 2), :] = _pk(q[:, c0:c0 + 128])
            q_s[9 + t, pl.ds(rh, R // 2), :] = _pk(pltpu.roll(q[:, c0:c0 + 128], 64, 1))
        yield
        yield
        k = jnp.dot(xn, wqkv_ref[:, D:2 * D], preferred_element_type=F32)
        for t in range(9):
            c0 = 128 * t if t < 5 else 64 + 128 * (t - 5)
            k_s[t, pl.ds(rh + W // 2, R // 2), :] = _pk(k[:, c0:c0 + 128])
            k_s[9 + t, pl.ds(rh + W // 2, R // 2), :] = _pk(pltpu.roll(k[:, c0:c0 + 128], 64, 1))
        yield
        yield
        vt = lax.dot_general(wvt_s[...], xn, NT, preferred_element_type=F32)
        vt = jnp.concatenate([vt, jnp.zeros((8, R), F32)], axis=0)
        row = lax.broadcasted_iota(jnp.int32, (32, R), 0)
        for h in range(H):
            w0 = 40 * (h // 2) + 16 * (h % 2)
            one = 0 if h % 2 else 24
            blk = jnp.where(row == one, 1.0, vt[w0:w0 + 32, :])
            vt_s[h, :, pl.ds(r0 + W, R)] = _pk(blk)

    def attn_tile(i, half, edge):
        q0 = i * T if edge else pl.multiple_of(i * T, T)
        sk = (2 - i) if edge else 0
        kk = lax.broadcasted_iota(jnp.int32, (T, T), 0)
        qq = lax.broadcasted_iota(jnp.int32, (T, T), 1)
        upper = kk > qq
        use2 = ((kk < T // 2) == (qq < T // 2)) & (upper == (kk >= T // 2))
        lane = lax.broadcasted_iota(jnp.int32, (T, 128), 1)
        sub = lax.broadcasted_iota(jnp.int32, (8, T), 0)
        q2 = i * (T // 2) if edge else pl.multiple_of(i * (T // 2), T // 2)

        def scores(h):
            t, off = _head_tile(h)
            if not edge:
                hq = T // 4
                la = (lane[:hq] >= off) & (lane[:hq] < off + DH)
                lb = (((lane[:hq] + 64) & 127) >= off) & (((lane[:hq] + 64) & 127) < off + DH)
                la2 = jnp.concatenate([la, la], axis=0)
                qm = jnp.concatenate([
                    jnp.where(la, q_s[t, pl.ds(q2, hq), :], 0),
                    jnp.where(lb, q_s[9 + t, pl.ds(q2 + hq, hq), :], 0)], axis=0)
                ld = lambda c, r, n: k_s[t + 9 * c, pl.ds(q2 + r, n), :]
                k1 = jnp.where(la2, ld(0, 0, 2 * hq), ld(1, 4 * hq, 2 * hq))
                k2 = jnp.where(la, ld(0, 4 * hq, hq), ld(1, hq, hq))
                kb = jnp.where(la2, ld(0, 2 * hq, 2 * hq), ld(1, 2 * hq, 2 * hq))
                return lax.dot_general(_up(jnp.concatenate([k1, kb, k2], axis=0)), _up(qm), NT,
                                       preferred_element_type=F32)
            qt = _up(q_s[t, pl.ds(q2, T // 2), :])
            qm = jnp.where((lane >= off) & (lane < off + DH), qt, jnp.zeros_like(qt))
            kt = _up(k_s[t, pl.ds(q2 + sk * T // 2, (3 - sk) * T // 2), :])
            return lax.dot_general(kt, qm, NT, preferred_element_type=F32)

        def probs(s):
            if edge:
                sc = jnp.where(upper, -1e9, s[-T:])
                sall = sc if sk == 2 else jnp.concatenate([s[0:T], sc], axis=0)
                return jnp.exp2(sall - jnp.max(sall, axis=0, keepdims=True)).astype(BF)
            s1, sb, s2 = s[0:T], s[T:2 * T], s[2 * T:]
            sm = jnp.concatenate([jnp.where(use2[:T // 2], s2, s1[:T // 2]),
                                  jnp.where(use2[T // 2:], s2, s1[T // 2:])], axis=0)
            mx = jnp.max(jnp.maximum(sm, sb), axis=0, keepdims=True)
            pm = jnp.exp2(sm - mx)
            pb = jnp.exp2(sb - mx).astype(BF)
            pa = jnp.where(upper, pm, 0.0).astype(BF)
            pc = jnp.where(upper, 0.0, pm).astype(BF)
            return jnp.concatenate([pa, pb, pc], axis=0)

        def pv(h, p):
            return jnp.dot(_up(vt_s[h, :, pl.ds(q0 + sk * T, (3 - sk) * T)]), p, preferred_element_type=F32)

        G = 4
        ss = [scores(h) for h in range(G)]
        for g0 in range(0, H, G):
            ps = [probs(s) for s in ss]
            if g0 + G < H:
                ss = [scores(h) for h in range(g0 + G, g0 + 2 * G)]
            os_ = [pv(g0 + u, ps[u]) for u in range(G)]
            yield
            for u in range(0, G, 2):
                oe, oo = os_[u], os_[u + 1]
                prev = oe[0:24] * (1.0 / oe[24:25])
                on = oo * (1.0 / oo[0:1])
                mid = jnp.where(sub < 4, prev[16:24], on[0:8])
                b0 = 20 * (g0 + u)
                ot_s[(i // 2) % 2, b0:b0 + 40, pl.ds(half * T, T)] = jnp.concatenate(
                    [prev[0:16], mid, on[8:24]], axis=0)

    def attn(j, edge):
        for half in range(2):
            yield from attn_tile(2 * j + half, half, edge)

    def run(*gens):
        gens = list(gens)
        while gens:
            for g in list(gens):
                try:
                    next(g)
                except StopIteration:
                    gens.remove(g)

    def ffn(j, last):
        r0 = j * R if isinstance(j, int) else pl.multiple_of(j * R, R)
        o = ot_s[j % 2].T.astype(BF)
        x = xs[pl.ds(r0, R), :] + jnp.dot(o, wo_ref[...], preferred_element_type=F32)
        xn = _ln(x).astype(BF)
        xs[pl.ds(r0, R), :] = x
        yield
        for c0 in range(0, F, FC):
            c1 = min(F, c0 + FC)
            hh = lax.dot_general(xn, w1_ref[c0:c1, :], NT, preferred_element_type=F32)
            hh = hh + b1_ref[:, c0:c1].astype(F32)
            g_s[:, c0:c1] = _pk(jax.nn.gelu(hh, approximate=True))
            yield
        for c0 in range(0, D, NC):
            c1 = c0 + NC
            y = (xs[pl.ds(r0, R), c0:c1] + b2_ref[:, c0:c1].astype(F32)
                 + jnp.dot(_up(g_s[...]), w2_ref[:, c0:c1], preferred_element_type=F32))
            if last:
                o_ref[pl.ds(r0, R), c0:c1] = y.astype(o_ref.dtype)
            else:
                xs[pl.ds(r0, R), c0:c1] = y
            yield

    for layer in range(2):
        if layer == 0:
            xcp[0].wait()
            run(qkv(0, True))
            xcp[1].wait()
        else:
            run(ffn(NB - 1, False), qkv(0, False))
        run(attn(0, True), qkv(1, layer == 0))
        if layer == 0:
            xcp[2].wait()

        def p1(j, c):
            run(qkv(j, layer == 0))
            return c
        lax.fori_loop(2, NB, p1, 0)
        if layer == 0:
            for c in cps[2:]:
                c.wait()

        def p2(j, c):
            run(attn(j, False), ffn(j - 1, layer == 1))
            return c
        if layer == 0:
            lax.fori_loop(1, NB, p2, 0)
        else:
            lax.fori_loop(1, NB // 2 + 1, p2, 0)
            ocp[0].start()
            lax.fori_loop(NB // 2 + 1, NB, p2, 0)
            run(ffn(NB - 1, True))
    ocp[1].start()
    ocp[0].wait()
    ocp[1].wait()


@jax.jit
def pallas_interleave_layers__sliding_block__dense_activation_gelu__prompt_kernel(
    A_x, A_wqkv, A_wo, B_x, B_w1, B_b1, B_w2, B_b2,
):
    hb = pl.BlockSpec(memory_space=pl.ANY)
    vm = pl.BlockSpec(memory_space=pltpu.VMEM)
    out = pl.pallas_call(
        _kernel,
        out_shape=jax.ShapeDtypeStruct((S, D), A_x.dtype),
        in_specs=[hb, hb, hb, hb, vm, hb, vm],
        out_specs=hb,
        scratch_shapes=[
            pltpu.VMEM((S, D), F32),
            pltpu.VMEM((18, S // 2, 128), I32),
            pltpu.VMEM((18, (S + W) // 2, 128), I32),
            pltpu.VMEM((H, 16, S + W), I32),
            pltpu.VMEM((D, D), BF),
            pltpu.VMEM((2, D, R), F32),
            pltpu.VMEM((S, D), BF), pltpu.VMEM((D, 3 * D), BF), pltpu.VMEM((D, D), BF),
            pltpu.VMEM((F, D), BF), pltpu.VMEM((F, D), BF), pltpu.VMEM((S, D), BF),
            pltpu.VMEM((R // 2, F), I32),
            pltpu.SemaphoreType.DMA((9,)),
        ],
        compiler_params=pltpu.CompilerParams(vmem_limit_bytes=100 * 1024 * 1024),
    )(A_x.reshape(S, D), A_wqkv, A_wo, B_w1.T, B_b1.reshape(1, F), B_w2, B_b2.reshape(1, D))
    return out.reshape(1, S, D)
```

```python
import math
import jax
import jax.numpy as jnp
from jax import lax
import jax.experimental.pallas as pl
import jax.experimental.pallas.tpu as pltpu

S, D, H, DH, W, F = 2048, 640, 32, 20, 256, 1728
T = 128
R = 256
NB = S // R
FC = 128
NC = 128
NT = (((1,), (1,)), ((), ()))
BF = jnp.bfloat16
F32 = jnp.float32
I32 = jnp.int32
_pk = lambda v: pltpu.bitcast(v.astype(BF), I32)
_up = lambda v: pltpu.bitcast(v, BF)
QSCALE = (DH ** -0.5) * math.log2(math.e)


def _ln(x):
    m = jnp.mean(x, axis=-1, keepdims=True)
    c = x - m
    v = jnp.mean(c * c, axis=-1, keepdims=True)
    return c * lax.rsqrt(v + 1e-5)


def _head_tile(h):
    lo, hi = DH * h, DH * h + DH - 1
    if lo // 128 == hi // 128:
        return lo // 128, lo % 128
    t = (lo - 64) // 128
    return 5 + t, lo - 64 - 128 * t


def _kernel(x_h, wqkv_h, wo_h, w1_h, b1_ref, w2_h, b2_ref, o_h,
            xs, q_s, k_s, vt_s, wvt_s, ot_s, x_ref, wqkv_ref, wo_ref, w1_ref, w2_ref, o_ref, g_s, sems):
    cps = [pltpu.make_async_copy(a, b, sems.at[n]) for n, (a, b) in enumerate(
        [(wqkv_h, wqkv_ref), (x_h.at[0:R], x_ref.at[0:R]), (wo_h, wo_ref), (w1_h, w1_ref), (w2_h, w2_ref)])]
    xcp = [cps[1],
           pltpu.make_async_copy(x_h.at[R:2 * R], x_ref.at[R:2 * R], sems.at[7]),
           pltpu.make_async_copy(x_h.at[2 * R:S], x_ref.at[2 * R:S], sems.at[8])]
    for c in cps[:2] + xcp[1:] + cps[2:]:
        c.start()
    ocp = [pltpu.make_async_copy(o_ref.at[lo:hi], o_h.at[lo:hi], sems.at[n])
           for n, lo, hi in ((5, 0, S // 2), (6, S // 2, S - R), (9, S - R, S))]

    cps[0].wait()
    wvt_s[...] = wqkv_ref[:, 2 * D:].astype(F32).T.astype(BF)
    k_s[:, 0:W // 2, :] = jnp.zeros((18, W // 2, 128), I32)
    vt_s[:, :, 0:W] = jnp.zeros((H, 16, W), I32)


    def qkv(j, first):
        r0 = j * R if isinstance(j, int) else pl.multiple_of(j * R, R)
        rh = j * (R // 2) if isinstance(j, int) else pl.multiple_of(j * (R // 2), R // 2)
        if first:
            x = x_ref[pl.ds(r0, R), :].astype(F32)
            xs[pl.ds(r0, R), :] = x
        else:
            x = xs[pl.ds(r0, R), :]
        xn = _ln(x).astype(BF)
        q = jnp.dot(xn, wqkv_ref[:, 0:D], preferred_element_type=F32) * QSCALE
        for t in range(9):
            c0 = 128 * t if t < 5 else 64 + 128 * (t - 5)
            q_s[t, pl.ds(rh, R // 2), :] = _pk(q[:, c0:c0 + 128])
            q_s[9 + t, pl.ds(rh, R // 2), :] = _pk(pltpu.roll(q[:, c0:c0 + 128], 64, 1))
        yield
        yield
        k = jnp.dot(xn, wqkv_ref[:, D:2 * D], preferred_element_type=F32)
        for t in range(9):
            c0 = 128 * t if t < 5 else 64 + 128 * (t - 5)
            k_s[t, pl.ds(rh + W // 2, R // 2), :] = _pk(k[:, c0:c0 + 128])
            k_s[9 + t, pl.ds(rh + W // 2, R // 2), :] = _pk(pltpu.roll(k[:, c0:c0 + 128], 64, 1))
        yield
        yield
        vt = lax.dot_general(wvt_s[...], xn, NT, preferred_element_type=F32)
        vt = jnp.concatenate([vt, jnp.zeros((8, R), F32)], axis=0)
        row = lax.broadcasted_iota(jnp.int32, (32, R), 0)
        for h in range(H):
            w0 = 40 * (h // 2) + 16 * (h % 2)
            one = 0 if h % 2 else 24
            blk = jnp.where(row == one, 1.0, vt[w0:w0 + 32, :])
            vt_s[h, :, pl.ds(r0 + W, R)] = _pk(blk)

    def attn_tile(i, half, edge):
        q0 = i * T if isinstance(i, int) else pl.multiple_of(i * T, T)
        sk = (2 - i) if edge else 0
        kk = lax.broadcasted_iota(jnp.int32, (T, T), 0)
        qq = lax.broadcasted_iota(jnp.int32, (T, T), 1)
        upper = kk > qq
        use2 = ((kk < T // 2) == (qq < T // 2)) & (upper == (kk >= T // 2))
        lane = lax.broadcasted_iota(jnp.int32, (T, 128), 1)
        sub = lax.broadcasted_iota(jnp.int32, (8, T), 0)
        q2 = i * (T // 2) if isinstance(i, int) else pl.multiple_of(i * (T // 2), T // 2)

        def scores(h):
            t, off = _head_tile(h)
            if not edge:
                hq = T // 4
                la = (lane[:hq] >= off) & (lane[:hq] < off + DH)
                lb = (((lane[:hq] + 64) & 127) >= off) & (((lane[:hq] + 64) & 127) < off + DH)
                la2 = jnp.concatenate([la, la], axis=0)
                qm = jnp.concatenate([
                    jnp.where(la, q_s[t, pl.ds(q2, hq), :], 0),
                    jnp.where(lb, q_s[9 + t, pl.ds(q2 + hq, hq), :], 0)], axis=0)
                ld = lambda c, r, n: k_s[t + 9 * c, pl.ds(q2 + r, n), :]
                k1 = jnp.where(la2, ld(0, 0, 2 * hq), ld(1, 4 * hq, 2 * hq))
                k2 = jnp.where(la, ld(0, 4 * hq, hq), ld(1, hq, hq))
                kb = jnp.where(la2, ld(0, 2 * hq, 2 * hq), ld(1, 2 * hq, 2 * hq))
                return lax.dot_general(_up(jnp.concatenate([k1, kb, k2], axis=0)), _up(qm), NT,
                                       preferred_element_type=F32)
            qt = _up(q_s[t, pl.ds(q2, T // 2), :])
            qm = jnp.where((lane >= off) & (lane < off + DH), qt, jnp.zeros_like(qt))
            kt = _up(k_s[t, pl.ds(q2 + sk * T // 2, (3 - sk) * T // 2), :])
            return lax.dot_general(kt, qm, NT, preferred_element_type=F32)

        def probs(s):
            if edge:
                sc = jnp.where(upper, -1e9, s[-T:])
                sall = sc if sk == 2 else jnp.concatenate([s[0:T], sc], axis=0)
                return jnp.exp2(sall - jnp.max(sall, axis=0, keepdims=True)).astype(BF)
            s1, sb, s2 = s[0:T], s[T:2 * T], s[2 * T:]
            sm = jnp.concatenate([jnp.where(use2[:T // 2], s2, s1[:T // 2]),
                                  jnp.where(use2[T // 2:], s2, s1[T // 2:])], axis=0)
            mx = jnp.max(jnp.maximum(sm, sb), axis=0, keepdims=True)
            pm = jnp.exp2(sm - mx)
            pb = jnp.exp2(sb - mx).astype(BF)
            pmb = pm.astype(BF)
            pa = jnp.where(upper, pmb, jnp.zeros_like(pmb))
            pc = jnp.where(upper, jnp.zeros_like(pmb), pmb)
            return jnp.concatenate([pa, pb, pc], axis=0)

        def pv(h, p):
            return jnp.dot(_up(vt_s[h, :, pl.ds(q0 + sk * T, (3 - sk) * T)]), p, preferred_element_type=F32)

        G = 4
        ss = [scores(h) for h in range(G)]
        for g0 in range(0, H, G):
            ps = [probs(s) for s in ss]
            if g0 + G < H:
                ss = [scores(h) for h in range(g0 + G, g0 + 2 * G)]
            os_ = [pv(g0 + u, ps[u]) for u in range(G)]
            yield
            for u in range(0, G, 2):
                oe, oo = os_[u], os_[u + 1]
                prev = oe[0:24] * (1.0 / oe[24:25])
                on = oo * (1.0 / oo[0:1])
                mid = jnp.where(sub < 4, prev[16:24], on[0:8])
                b0 = 20 * (g0 + u)
                ot_s[(i // 2) % 2, b0:b0 + 40, pl.ds(half * T, T)] = jnp.concatenate(
                    [prev[0:16], mid, on[8:24]], axis=0)

    def attn(j, edge):
        for half in range(2):
            yield from attn_tile(2 * j + half, half, edge)

    def run(*gens):
        gens = list(gens)
        while gens:
            for g in list(gens):
                try:
                    next(g)
                except StopIteration:
                    gens.remove(g)

    def ffn(j, last):
        r0 = j * R if isinstance(j, int) else pl.multiple_of(j * R, R)
        o = ot_s[j % 2].T.astype(BF)
        x = xs[pl.ds(r0, R), :] + jnp.dot(o, wo_ref[...], preferred_element_type=F32)
        xn = _ln(x).astype(BF)
        xs[pl.ds(r0, R), :] = x
        yield
        for c0 in range(0, F, FC):
            c1 = min(F, c0 + FC)
            hh = lax.dot_general(xn, w1_ref[c0:c1, :], NT, preferred_element_type=F32)
            hh = hh + b1_ref[:, c0:c1].astype(F32)
            g_s[:, c0:c1] = _pk(jax.nn.gelu(hh, approximate=True))
            yield
        for c0 in range(0, D, NC):
            c1 = c0 + NC
            y = (xs[pl.ds(r0, R), c0:c1] + b2_ref[:, c0:c1].astype(F32)
                 + jnp.dot(_up(g_s[...]), w2_ref[:, c0:c1], preferred_element_type=F32))
            if last:
                o_ref[pl.ds(r0, R), c0:c1] = y.astype(o_ref.dtype)
            else:
                xs[pl.ds(r0, R), c0:c1] = y
            yield

    for layer in range(2):
        if layer == 0:
            xcp[0].wait()
            run(qkv(0, True))
            xcp[1].wait()
        else:
            run(ffn(NB - 1, False), qkv(0, False))
        run(attn(0, True), qkv(1, layer == 0))
        if layer == 0:
            xcp[2].wait()
            for c in cps[2:]:
                c.wait()

        def p2(j, c):
            if layer == 1:
                pl.when(j == NB // 2 + 1)(ocp[0].start)
            run(attn(j, False), ffn(j - 1, layer == 1), qkv(j + 1, layer == 0))
            return c
        lax.fori_loop(1, NB - 1, p2, 0)
        run(attn(NB - 1, False), ffn(NB - 2, layer == 1))
        if layer == 1:
            ocp[1].start()
            run(ffn(NB - 1, True))
    ocp[2].start()
    for c in ocp:
        c.wait()


@jax.jit
def pallas_interleave_layers__sliding_block__dense_activation_gelu__prompt_kernel(
    A_x, A_wqkv, A_wo, B_x, B_w1, B_b1, B_w2, B_b2,
):
    hb = pl.BlockSpec(memory_space=pl.ANY)
    vm = pl.BlockSpec(memory_space=pltpu.VMEM)
    out = pl.pallas_call(
        _kernel,
        out_shape=jax.ShapeDtypeStruct((S, D), A_x.dtype),
        in_specs=[hb, hb, hb, hb, vm, hb, vm],
        out_specs=hb,
        scratch_shapes=[
            pltpu.VMEM((S, D), F32),
            pltpu.VMEM((18, S // 2, 128), I32),
            pltpu.VMEM((18, (S + W) // 2, 128), I32),
            pltpu.VMEM((H, 16, S + W), I32),
            pltpu.VMEM((D, D), BF),
            pltpu.VMEM((2, D, R), F32),
            pltpu.VMEM((S, D), BF), pltpu.VMEM((D, 3 * D), BF), pltpu.VMEM((D, D), BF),
            pltpu.VMEM((F, D), BF), pltpu.VMEM((F, D), BF), pltpu.VMEM((S, D), BF),
            pltpu.VMEM((R // 2, F), I32),
            pltpu.SemaphoreType.DMA((10,)),
        ],
        compiler_params=pltpu.CompilerParams(vmem_limit_bytes=100 * 1024 * 1024),
    )(A_x.reshape(S, D), A_wqkv, A_wo, B_w1.T, B_b1.reshape(1, F), B_w2, B_b2.reshape(1, D))
    return out.reshape(1, S, D)
```

```python
import math
import jax
import jax.numpy as jnp
from jax import lax
import jax.experimental.pallas as pl
import jax.experimental.pallas.tpu as pltpu

S, D, H, DH, W, F = 2048, 640, 32, 20, 256, 1728
T = 128
R = 256
NB = S // R
FC = 128
NC = 128
NT = (((1,), (1,)), ((), ()))
BF = jnp.bfloat16
F32 = jnp.float32
I32 = jnp.int32
_pk = lambda v: pltpu.bitcast(v.astype(BF), I32)
_up = lambda v: pltpu.bitcast(v, BF)
QSCALE = (DH ** -0.5) * math.log2(math.e)


def _ln(x):
    m = jnp.mean(x, axis=-1, keepdims=True)
    c = x - m
    v = jnp.mean(c * c, axis=-1, keepdims=True)
    return c * lax.rsqrt(v + 1e-5)


def _head_tile(h):
    lo, hi = DH * h, DH * h + DH - 1
    if lo // 128 == hi // 128:
        return lo // 128, lo % 128
    t = (lo - 64) // 128
    return 5 + t, lo - 64 - 128 * t


def _kernel(x_h, wqkv_h, wo_h, w1_h, b1_ref, w2_h, b2_ref, o_h,
            xs, q_s, k_s, vt_s, wvt_s, ot_s, x_ref, wqkv_ref, wo_ref, w1_ref, w2_ref, o_ref, g_s, sems):
    cps = [pltpu.make_async_copy(a, b, sems.at[n]) for n, (a, b) in enumerate(
        [(wqkv_h, wqkv_ref), (x_h.at[0:R], x_ref.at[0:R]), (wo_h, wo_ref), (w1_h, w1_ref), (w2_h, w2_ref)])]
    xcp = [cps[1],
           pltpu.make_async_copy(x_h.at[R:2 * R], x_ref.at[R:2 * R], sems.at[7]),
           pltpu.make_async_copy(x_h.at[2 * R:S], x_ref.at[2 * R:S], sems.at[8])]
    for c in cps[:2] + xcp[1:] + cps[2:]:
        c.start()
    ocp = [pltpu.make_async_copy(o_ref.at[lo:hi], o_h.at[lo:hi], sems.at[n])
           for n, lo, hi in ((5, 0, S // 2), (6, S // 2, S - R), (9, S - R, S))]

    cps[0].wait()
    wvt_s[...] = wqkv_ref[:, 2 * D:].astype(F32).T.astype(BF)
    k_s[:, 0:W // 2, :] = jnp.zeros((H, W // 2, 128), I32)
    vt_s[:, :, 0:W] = jnp.zeros((H, 16, W), I32)


    def qkv(j, first):
        r0 = j * R if isinstance(j, int) else pl.multiple_of(j * R, R)
        rh = j * (R // 2) if isinstance(j, int) else pl.multiple_of(j * (R // 2), R // 2)
        if first:
            x = x_ref[pl.ds(r0, R), :].astype(F32)
            xs[pl.ds(r0, R), :] = x
        else:
            x = xs[pl.ds(r0, R), :]
        xn = _ln(x).astype(BF)
        q = jnp.dot(xn, wqkv_ref[:, 0:D], preferred_element_type=F32) * QSCALE
        lane = lax.broadcasted_iota(I32, (16, 128), 1)
        for t in range(9):
            c0 = 128 * t if t < 5 else 64 + 128 * (t - 5)
            qp = _pk(q[:, c0:c0 + 128])
            qc = [qp] + [pltpu.roll(qp, 32 * c, 1) for c in range(1, 4)]
            for h in range(H):
                if _head_tile(h)[0] == t:
                    rel = (lane - _head_tile(h)[1]) & 127
                    q_s[h, pl.ds(rh, R // 2), :] = jnp.concatenate(
                        [jnp.where((rel >= 32 * (g % 4)) & (rel < 32 * (g % 4) + DH),
                                   qc[g % 4][16 * g:16 * g + 16], 0) for g in range(R // 32)], axis=0)
        yield
        yield
        k = jnp.dot(xn, wqkv_ref[:, D:2 * D], preferred_element_type=F32)
        lane = lax.broadcasted_iota(I32, (R // 2, 128), 1)
        for t in range(9):
            c0 = 128 * t if t < 5 else 64 + 128 * (t - 5)
            kp = _pk(k[:, c0:c0 + 128])
            kc = [kp] + [pltpu.roll(kp, 32 * c, 1) for c in range(1, 4)]
            for h in range(H):
                if _head_tile(h)[0] == t:
                    sl = ((lane - _head_tile(h)[1]) & 127) >> 5
                    k_s[h, pl.ds(rh + W // 2, R // 2), :] = jnp.where(
                        sl == 0, kc[0], jnp.where(sl == 1, kc[1], jnp.where(sl == 2, kc[2], kc[3])))
        yield
        yield
        vt = lax.dot_general(wvt_s[...], xn, NT, preferred_element_type=F32)
        vt = jnp.concatenate([vt, jnp.zeros((8, R), F32)], axis=0)
        row = lax.broadcasted_iota(jnp.int32, (32, R), 0)
        for h in range(H):
            w0 = 40 * (h // 2) + 16 * (h % 2)
            one = 0 if h % 2 else 24
            blk = jnp.where(row == one, 1.0, vt[w0:w0 + 32, :])
            vt_s[h, :, pl.ds(r0 + W, R)] = _pk(blk)

    def attn_tile(i, half, edge):
        q0 = i * T if isinstance(i, int) else pl.multiple_of(i * T, T)
        sk = (2 - i) if edge else 0
        kk = lax.broadcasted_iota(jnp.int32, (T, T), 0)
        qq = lax.broadcasted_iota(jnp.int32, (T, T), 1)
        upper = kk > qq
        use2 = ((kk >> 5) == (qq >> 5)) & (kk <= qq)
        lane = lax.broadcasted_iota(jnp.int32, (T, 128), 1)
        sub = lax.broadcasted_iota(jnp.int32, (8, T), 0)
        q2 = i * (T // 2) if isinstance(i, int) else pl.multiple_of(i * (T // 2), T // 2)

        def scores(h):
            t, off = _head_tile(h)
            qm = _up(q_s[h, pl.ds(q2, T // 2), :])
            if edge:
                kt = k_s[h, pl.ds(q2 + sk * T // 2, (3 - sk) * T // 2), :]
            else:
                sl = ((lane[:T // 2] - off) & 127) >> 5
                rb = lax.broadcasted_iota(I32, (T // 2, 128), 0) >> 4
                ka = k_s[h, pl.ds(q2, T // 2), :]
                kb = k_s[h, pl.ds(q2 + T // 2, T // 2), :]
                kc = k_s[h, pl.ds(q2 + T, T // 2), :]
                s16 = sl[:16]
                k2 = jnp.where(s16 == 0, kc[0:16], jnp.where(s16 == 1, kc[16:32],
                               jnp.where(s16 == 2, kc[32:48], kc[48:64])))
                kt = jnp.concatenate([jnp.where(sl <= rb, ka, kc), kb, k2], axis=0)
            return lax.dot_general(_up(kt), qm, NT, preferred_element_type=F32)

        def probs(s):
            if edge:
                sc = jnp.where(upper, -1e9, s[-T:])
                sall = sc if sk == 2 else jnp.concatenate([s[0:T], sc], axis=0)
                return jnp.exp2(sall - jnp.max(sall, axis=0, keepdims=True)).astype(BF)
            s1, sb, s2 = s[0:T], s[T:2 * T], s[2 * T:]
            sm = jnp.where(use2, jnp.concatenate([s2] * 4, axis=0), s1)
            mx = jnp.max(jnp.maximum(sm, sb), axis=0, keepdims=True)
            pm = jnp.exp2(sm - mx)
            pb = jnp.exp2(sb - mx).astype(BF)
            pmb = pm.astype(BF)
            pa = jnp.where(upper, pmb, jnp.zeros_like(pmb))
            pc = jnp.where(upper, jnp.zeros_like(pmb), pmb)
            return jnp.concatenate([pa, pb, pc], axis=0)

        def pv(h, p):
            return jnp.dot(_up(vt_s[h, :, pl.ds(q0 + sk * T, (3 - sk) * T)]), p, preferred_element_type=F32)

        G = 4
        ss = [scores(h) for h in range(G)]
        for g0 in range(0, H, G):
            ps = [probs(s) for s in ss]
            if g0 + G < H:
                ss = [scores(h) for h in range(g0 + G, g0 + 2 * G)]
            os_ = [pv(g0 + u, ps[u]) for u in range(G)]
            yield
            for u in range(0, G, 2):
                oe, oo = os_[u], os_[u + 1]
                prev = oe[0:24] * (1.0 / oe[24:25])
                on = oo * (1.0 / oo[0:1])
                mid = jnp.where(sub < 4, prev[16:24], on[0:8])
                b0 = 20 * (g0 + u)
                ot_s[(i // 2) % 2, b0:b0 + 40, pl.ds(half * T, T)] = jnp.concatenate(
                    [prev[0:16], mid, on[8:24]], axis=0)

    def attn(j, edge):
        for half in range(2):
            yield from attn_tile(2 * j + half, half, edge)

    def run(*gens):
        gens = list(gens)
        while gens:
            for g in list(gens):
                try:
                    next(g)
                except StopIteration:
                    gens.remove(g)

    def ffn(j, last):
        r0 = j * R if isinstance(j, int) else pl.multiple_of(j * R, R)
        o = ot_s[j % 2].T.astype(BF)
        x = xs[pl.ds(r0, R), :] + jnp.dot(o, wo_ref[...], preferred_element_type=F32)
        xn = _ln(x).astype(BF)
        xs[pl.ds(r0, R), :] = x
        yield
        for c0 in range(0, F, FC):
            c1 = min(F, c0 + FC)
            hh = lax.dot_general(xn, w1_ref[c0:c1, :], NT, preferred_element_type=F32)
            hh = hh + b1_ref[:, c0:c1].astype(F32)
            g_s[:, c0:c1] = _pk(jax.nn.gelu(hh, approximate=True))
            yield
        for c0 in range(0, D, NC):
            c1 = c0 + NC
            y = (xs[pl.ds(r0, R), c0:c1] + b2_ref[:, c0:c1].astype(F32)
                 + jnp.dot(_up(g_s[...]), w2_ref[:, c0:c1], preferred_element_type=F32))
            if last:
                o_ref[pl.ds(r0, R), c0:c1] = y.astype(o_ref.dtype)
            else:
                xs[pl.ds(r0, R), c0:c1] = y
            yield

    for layer in range(2):
        if layer == 0:
            xcp[0].wait()
            run(qkv(0, True))
            xcp[1].wait()
        else:
            run(ffn(NB - 1, False), qkv(0, False))
        run(attn(0, True), qkv(1, layer == 0))
        if layer == 0:
            xcp[2].wait()
            for c in cps[2:]:
                c.wait()

        def p2(j, c):
            if layer == 1:
                pl.when(j == NB // 2 + 1)(ocp[0].start)
            run(attn(j, False), ffn(j - 1, layer == 1), qkv(j + 1, layer == 0))
            return c
        lax.fori_loop(1, NB - 1, p2, 0)
        run(attn(NB - 1, False), ffn(NB - 2, layer == 1))
        if layer == 1:
            ocp[1].start()
            run(ffn(NB - 1, True))
    ocp[2].start()
    for c in ocp:
        c.wait()


@jax.jit
def pallas_interleave_layers__sliding_block__dense_activation_gelu__prompt_kernel(
    A_x, A_wqkv, A_wo, B_x, B_w1, B_b1, B_w2, B_b2,
):
    hb = pl.BlockSpec(memory_space=pl.ANY)
    vm = pl.BlockSpec(memory_space=pltpu.VMEM)
    out = pl.pallas_call(
        _kernel,
        out_shape=jax.ShapeDtypeStruct((S, D), A_x.dtype),
        in_specs=[hb, hb, hb, hb, vm, hb, vm],
        out_specs=hb,
        scratch_shapes=[
            pltpu.VMEM((S, D), F32),
            pltpu.VMEM((H, S // 2, 128), I32),
            pltpu.VMEM((H, (S + W) // 2, 128), I32),
            pltpu.VMEM((H, 16, S + W), I32),
            pltpu.VMEM((D, D), BF),
            pltpu.VMEM((2, D, R), F32),
            pltpu.VMEM((S, D), BF), pltpu.VMEM((D, 3 * D), BF), pltpu.VMEM((D, D), BF),
            pltpu.VMEM((F, D), BF), pltpu.VMEM((F, D), BF), pltpu.VMEM((S, D), BF),
            pltpu.VMEM((R // 2, F), I32),
            pltpu.SemaphoreType.DMA((10,)),
        ],
        compiler_params=pltpu.CompilerParams(vmem_limit_bytes=100 * 1024 * 1024),
    )(A_x.reshape(S, D), A_wqkv, A_wo, B_w1.T, B_b1.reshape(1, F), B_w2, B_b2.reshape(1, D))
    return out.reshape(1, S, D)
```
